```python
import os as _os
_os.environ.setdefault("JAX_PLATFORMS", "cpu")
import jax
import jax.numpy as jnp

def _softmax(x, axis=-1):
    return jax.nn.softmax(x, axis=axis)
def _gelu(x):
    return jax.nn.gelu(x, approximate=True)
def _silu(x):
    return jax.nn.silu(x)
def _sigmoid(x):
    return jax.nn.sigmoid(x)
def _layernorm(x, axis=-1, eps=1e-5):
    m = jnp.mean(x, axis=axis, keepdims=True)
    v = jnp.var(x, axis=axis, keepdims=True)
    return (x - m) / jnp.sqrt(v + eps)
def _scatter_add(tgt, idx, src, axis=0):
    return tgt.at[idx].add(src)
def _segment_sum(src, seg, n):
    return jax.ops.segment_sum(src, seg, n)
class _Rng:
    def __init__(self, key):
        self._k = key
    def _next(self):
        self._k, sub = jax.random.split(self._k)
        return sub
    def normal(self, shape):
        return jax.random.normal(self._next(), shape, dtype=jnp.bfloat16)
    def randint(self, lo, hi, shape):
        return jax.random.randint(self._next(), shape, lo, hi, dtype=jnp.int32)
    def uniform(self, shape, lo=0.0, hi=1.0):
        return jax.random.uniform(self._next(), shape, jnp.bfloat16, lo, hi)
    def permutation(self, n):
        return jax.random.permutation(self._next(), n)


kernel_name = 'sequential_preLN__ssm_conv_h3__mixer_channel_mlp__prompt'

def setup_inputs():
    _rng = _Rng(jax.random.key(int.from_bytes(__import__("os").urandom(4), "little")))
    _w = (lambda a: (lambda t: t.astype(jnp.bfloat16) if jnp.issubdtype(t.dtype, jnp.floating) else t)(jnp.asarray(a)))
    def _A_setup():
        B, S, D = 1, 2048, 448
        ks = 4
        return {
            "q": _w((lambda *s: _rng.normal(s) * 0.05)(B, S, D)),
            "k": _w((lambda *s: _rng.normal(s) * 0.05)(B, S, D)),
            "v": _w((lambda *s: _rng.normal(s) * 0.05)(B, S, D)),
            "shift_k": _w((lambda *s: _rng.normal(s) * 0.05)(D, ks) * 0.5),
            "ssm_k": _w((lambda *s: _rng.normal(s) * 0.05)(D, S) * (1.0 / S ** 0.5)),
            "ssm_D": _w((lambda *s: _rng.normal(s) * 0.05)(D)),
        }
    _A_in = _A_setup()

    def _B_setup():
        B, S, D, F = 1, 2048, 448, 1792
        return {
            "x": _w((lambda *s: _rng.normal(s) * 0.05)(B, S, D)),
            "w1": _w((lambda *s: _rng.normal(s) * 0.2)(D, F) * (D ** -0.5)),
            "b1": _w((lambda *s: _rng.normal(s) * 0.2)(F)),
            "w2": _w((lambda *s: _rng.normal(s) * 0.2)(F, D) * (F ** -0.5)),
            "b2": _w((lambda *s: _rng.normal(s) * 0.05)(D)),
        }
    _B_in = _B_setup()

    return {
        "A_q": _A_in["q"],
        "A_k": _A_in["k"],
        "A_v": _A_in["v"],
        "A_shift_k": _A_in["shift_k"],
        "A_ssm_k": _A_in["ssm_k"],
        "A_ssm_D": _A_in["ssm_D"],
        "B_x": _B_in["x"],
        "B_w1": _B_in["w1"],
        "B_b1": _B_in["b1"],
        "B_w2": _B_in["w2"],
        "B_b2": _B_in["b2"],
    }

def reference(A_q, A_k, A_v, A_shift_k, A_ssm_k, A_ssm_D, B_x, B_w1, B_b1, B_w2, B_b2):
    def _A_ref(q, k, v, shift_k, ssm_k, ssm_D):
        B, S, D = q.shape
        ks = shift_k.shape[-1]
        k_pad = jnp.pad(k, ((0, 0), (ks - 1, 0), (0, 0)))
        k_shift = jnp.zeros_like(k)
        for t in range(ks):
            k_shift = k_shift + k_pad[:, t:t + S, :] * shift_k[:, ks - 1 - t][None, None, :]
        kv = k_shift * v
        L = 2 * S
        kv_pad = jnp.pad(kv, ((0, 0), (0, S), (0, 0)))
        kf_pad = jnp.pad(ssm_k, ((0, 0), (0, S)))
        kv_f = (lambda x, axes=(-2,-1): jnp.fft.rfft2(x.astype(jnp.float32), axes=axes))(kv_pad[:, None, :, :], axes=(1, 2))
        kf_f = (lambda x, axes=(-2,-1): jnp.fft.rfft2(x.astype(jnp.float32), axes=axes))(kf_pad[:, None, :], axes=(1, 2))
        kf_f = (lambda x, *d: x.transpose(*d))(kf_f, 1, 2, 0)
        y_f = kv_f * kf_f[None, :, :, :]
        y = (lambda x, s, axes=(-2,-1): jnp.fft.irfft2(x, s=s, axes=axes).astype(jnp.bfloat16))(y_f, (1, L), axes=(1, 2))[:, 0, :S, :]
        y = y + kv * ssm_D[None, None, :]
        return q * y

    def _B_ref(x, w1, b1, w2, b2):
        y = _layernorm(x, axis=-1)
        h = _gelu(jnp.einsum("bsd,df->bsf", y, w1) + b1)
        return jnp.einsum("bsf,fd->bsd", h, w2) + b2

    x = A_q
    h = x + _A_ref(_layernorm(x, axis=-1), A_k, A_v, A_shift_k, A_ssm_k, A_ssm_D)
    h2 = h + _B_ref(_layernorm(h, axis=-1), B_w1, B_b1, B_w2, B_b2)
    return h2
```

```python
import numpy as np, jax, jax.numpy as jnp
import jax.experimental.pallas as pl
import jax.experimental.pallas.tpu as pltpu
S,D,F=2048,448,1792
L=128; NB=S//L
T=512; R=T//L; NS=S//T
f32=jnp.float32; bf=jnp.bfloat16
def consts():
    t=np.arange(L)[:,None]; f=np.arange(L)[None,:]
    th=2*np.pi*t*(f+.5)/(2*L)
    FW=np.concatenate([np.cos(th),-np.sin(th)],1)
    return np.concatenate([FW,FW.T/L],0*1+0) if 0 else (FW.astype(np.float32),(FW.T/L).astype(np.float32))
def ln(x):
    m=jnp.mean(x,0,keepdims=True); c=x-m
    return c*jax.lax.rsqrt(jnp.mean(c*c,0,keepdims=True)+1e-5)
def col(row,n):
    row=jnp.concatenate([row,jnp.zeros((1,n-row.shape[1]),f32)],1)
    return jnp.broadcast_to(row,(128,n)).T
def kern(x_h,k_h,v_h,ssm_h,w1_h,w2_h,sk_ref,sd_ref,b1_ref,b2_ref,fw_ref,fi_ref,o_h,
         x,k,v,ssm,w1,w2,w1t,o,G,U,hn,sem,osem):
    def cp(i,s):
        a,b=((k_h,k),(v_h,v),(ssm_h,ssm),(x_h,x))[i]
        return pltpu.make_async_copy(a.at[:,s*T:(s+1)*T],b.at[:,s*T:(s+1)*T],sem.at[i,s])
    c1=pltpu.make_async_copy(w1_h,w1,sem.at[4,0]); c2=pltpu.make_async_copy(w2_h,w2,sem.at[4,1])
    for i in range(4): cp(i,0).start()
    for i in range(4): cp(i,1).start()
    c1.start(); c2.start()
    for s in range(2,NS):
        for i in range(4): cp(i,s).start()
    sk=sk_ref[...].astype(f32)
    skc=[col(sk[j:j+1],512)[:D] for j in range(4)]
    sdc=col(sd_ref[...].astype(f32),512)[:D]; b2c=col(b2_ref[...].astype(f32),512)[:D]
    tile=lambda a:jnp.concatenate([a]*R,1)
    lane=jax.lax.broadcasted_iota(jnp.int32,(D,L),1)
    sg=(1-2*(lane&1)).astype(f32)
    fw=fw_ref[...]; fi=fi_ref[...]
    hn[0,D:512,:]=hn[1,D:512,:]=jnp.where(jax.lax.broadcasted_iota(jnp.int32,(512-D,T),0)==0,1.0,0.0).astype(bf)
    kprev=jnp.zeros((D,L),f32); Kp=jnp.zeros((D,2*L),f32)
    st=dict(kprev=kprev,Kp=Kp)
    def conv(s):
        kprev=st['kprev'];Kp=st['Kp']
        for i in range(4): cp(i,s).wait()
        kvs=[]
        for r in range(R):
            j=s*R+r; sl=slice(j*L,(j+1)*L)
            kc=k[:,sl].astype(f32)
            ks=kc*skc[0]
            for m in range(1,4):
                ks=ks+jnp.where(lane>=m,pltpu.roll(kc,m,1),pltpu.roll(kprev,m,1))*skc[m]
            kprev=kc
            kv=ks*v[:,sl].astype(f32); kvs.append(kv)
            U[j]=jnp.dot(kv.astype(bf),fw,preferred_element_type=f32)
            Kf=jnp.dot(ssm[:,sl],fw,preferred_element_type=f32)
            G[j,:,0:L]=Kf[:,0:L]-sg*Kp[:,L:]
            G[j,:,L:]=Kf[:,L:]+sg*Kp[:,0:L]
            Kp=Kf
        ys=[]
        for r in range(R):
            j=s*R+r
            zr=zi=None
            for i in range(j+1):
                gr=G[i,:,0:L];gi=G[i,:,L:];ur=U[j-i,:,0:L];ui=U[j-i,:,L:]
                a=gr*ur-gi*ui; b=gr*ui+gi*ur
                zr,zi=(a,b) if zr is None else (zr+a,zi+b)
            Z=jnp.concatenate([zr,zi],1).astype(bf)
            ys.append(jnp.dot(Z,fi,preferred_element_type=f32)+kvs[r]*sdc)
        y=jnp.concatenate(ys,1)
        xs=x[:,s*T:(s+1)*T].astype(f32)
        h=xs+ln(xs)*y
        hn[s%2,0:D,:]=ln(h).astype(bf)
        st.update(kprev=kprev,Kp=Kp)
        return h
    def mlp(s,h):
        if s==0:
            c1.wait()
            for n in range(F//128):
                blk=jnp.concatenate([w1[:,n*128:(n+1)*128],b1_ref[:,n*128:(n+1)*128],jnp.zeros((63,128),bf)],0)
                w1t[n*128:(n+1)*128,:]=blk.T
            c2.wait()
        a=jnp.dot(w1t[...],hn[s%2],preferred_element_type=f32)
        g=jax.nn.gelu(a,approximate=True).astype(bf)
        oo=jnp.dot(w2[...],g,preferred_element_type=f32)+tile(b2c)
        o[:,s*T:(s+1)*T]=(h+oo).astype(bf)
        pltpu.make_async_copy(o.at[:,s*T:(s+1)*T],o_h.at[:,s*T:(s+1)*T],osem.at[s]).start()
    h=conv(0)
    for s in range(NS):
        h2=conv(s+1) if s+1<NS else None
        mlp(s,h); h=h2
    for s in range(NS):
        pltpu.make_async_copy(o.at[:,s*T:(s+1)*T],o_h.at[:,s*T:(s+1)*T],osem.at[s]).wait()
@jax.jit
def pallas_sequential_preLN__ssm_conv_h3__mixer_channel_mlp__prompt_kernel(A_q,A_k,A_v,A_shift_k,A_ssm_k,A_ssm_D,B_x,B_w1,B_b1,B_w2,B_b2):
    FW,FI=consts()
    any_=pl.BlockSpec(memory_space=pl.ANY); vm=pl.BlockSpec(memory_space=pltpu.VMEM)
    p5=lambda a:a
    V=pltpu.VMEM
    out=pl.pallas_call(kern,
      in_specs=[any_]*6+[vm]*6,
      out_specs=any_,out_shape=jax.ShapeDtypeStruct((D,S),bf),
      scratch_shapes=[V((D,S),bf)]*4+[V((D,F),bf),V((D,F),bf),V((F,512),bf),V((D,S),bf),
         V((NB,D,2*L),f32),V((NB,D,2*L),f32),V((2,512,T),bf),pltpu.SemaphoreType.DMA((5,NS)),pltpu.SemaphoreType.DMA((NS,))],
      compiler_params=pltpu.CompilerParams(vmem_limit_bytes=110*2**20),
    )(A_q[0].T,A_k[0].T,A_v[0].T,A_ssm_k,B_w1,B_w2.T,p5(A_shift_k.T),p5(A_ssm_D[None]),B_b1[None],p5(B_b2[None]),jnp.asarray(FW,bf),jnp.asarray(FI,bf))
    return out.T[None]
```
